```python
import os as _os
_os.environ.setdefault('JAX_PLATFORMS', 'cpu')
import jax
import jax.numpy as jnp

def _softmax(x, axis=-1):
    return jax.nn.softmax(x, axis=axis)

def _gelu(x):
    return jax.nn.gelu(x, approximate=True)

def _silu(x):
    return jax.nn.silu(x)

def _sigmoid(x):
    return jax.nn.sigmoid(x)

def _layernorm(x, axis=-1, eps=1e-05):
    m = jnp.mean(x, axis=axis, keepdims=True)
    v = jnp.var(x, axis=axis, keepdims=True)
    return (x - m) / jnp.sqrt(v + eps)

def _scatter_add(tgt, idx, src, axis=0):
    return tgt.at[idx].add(src)

def _segment_sum(src, seg, n):
    return jax.ops.segment_sum(src, seg, n)

class _Rng:

    def __init__(self, key):
        self._k = key

    def _next(self):
        self._k, sub = jax.random.split(self._k)
        return sub

    def normal(self, shape):
        return jax.random.normal(self._next(), shape, dtype=jnp.bfloat16)

    def randint(self, lo, hi, shape):
        return jax.random.randint(self._next(), shape, lo, hi, dtype=jnp.int32)

    def uniform(self, shape, lo=0.0, hi=1.0):
        return jax.random.uniform(self._next(), shape, jnp.bfloat16, lo, hi)

    def permutation(self, n):
        return jax.random.permutation(self._next(), n)
kernel_name = 'parallel_sum__memory_aug_recurrent_mem_tr__dense_activation_silu__prompt'

def setup_inputs():
    _rng = _Rng(jax.random.key(int.from_bytes(__import__("os").urandom(4), "little")))
    _w = lambda a: (lambda t: t.astype(jnp.bfloat16) if jnp.issubdtype(t.dtype, jnp.floating) else t)(jnp.asarray(a))

    def _A_setup():
        B, S, Dm = (1, 2048, 448)
        H, Dh = (16, 256)
        M, seg = (8, 32)
        seg = min(seg, S)
        S = S // seg * seg
        return {'x': _w((lambda *s: _rng.normal(s) * 0.05)(B, S, Dm)), 'mem0': _w((lambda *s: _rng.normal(s) * 0.2)(B, M, Dm)), 'Wq': _w((lambda *s: _rng.normal(s) * 0.8)(Dm, H, Dh) * Dm ** (-0.5)), 'Wk': _w((lambda *s: _rng.normal(s) * 0.8)(Dm, H, Dh) * Dm ** (-0.5)), 'Wv': _w((lambda *s: _rng.normal(s) * 0.2)(Dm, H, Dh) * Dm ** (-0.5)), 'Wo': _w((lambda *s: _rng.normal(s) * 0.2)(H, Dh, Dm) * (H * Dh) ** (-0.5)), 'seg_len': seg}
    _A_in = _A_setup()

    def _B_setup():
        B, S, D, F = (1, 2048, 448, 1792)
        return {'x': _w((lambda *s: _rng.normal(s) * 0.05)(B, S, D)), 'w1': _w((lambda *s: _rng.normal(s) * 0.05)(D, F) * D ** (-0.5)), 'w2': _w((lambda *s: _rng.normal(s) * 0.05)(F, D) * F ** (-0.5))}
    _B_in = _B_setup()
    return {'A_x': _A_in['x'], 'A_mem0': _A_in['mem0'], 'A_Wq': _A_in['Wq'], 'A_Wk': _A_in['Wk'], 'A_Wv': _A_in['Wv'], 'A_Wo': _A_in['Wo'], 'A_seg_len': _A_in['seg_len'], 'B_x': _B_in['x'], 'B_w1': _B_in['w1'], 'B_w2': _B_in['w2']}

def reference(A_x, A_mem0, A_Wq, A_Wk, A_Wv, A_Wo, A_seg_len, B_x, B_w1, B_w2):

    def _A_ref(x, mem0, Wq, Wk, Wv, Wo, seg_len):
        B, S, Dm = x.shape
        H, Dh = (Wq.shape[1], Wq.shape[2])
        M = mem0.shape[1]
        scale = Dh ** (-0.5)
        n_seg = S // seg_len
        L = M + seg_len
        idx = jnp.arange(L)
        mask = (idx[:, None] < M) | (idx[:, None] >= idx[None, :])
        mem = mem0
        outs = []
        for s in range(n_seg):
            xs = x[:, s * seg_len:(s + 1) * seg_len, :].copy()
            h = jnp.concatenate([mem, xs], axis=1)
            q = jnp.einsum('btd,dhe->bhte', h, Wq)
            k = jnp.einsum('btd,dhe->bhte', h, Wk)
            v = jnp.einsum('btd,dhe->bhte', h, Wv)
            scores = jnp.einsum('bhqe,bhke->bhqk', q, k) * scale
            scores = jnp.where(mask[None, None], scores, -1000000000.0)
            p = _softmax(scores, axis=-1)
            o = jnp.einsum('bhqk,bhke->bhqe', p, v)
            o = jnp.einsum('bhte,hed->btd', o, Wo)
            mem = o[:, :M, :].copy()
            outs.append(o[:, M:, :])
        return jnp.concatenate(outs, axis=1)

    def _B_ref(x, w1, w2):
        h = jnp.einsum('bsd,df->bsf', x, w1)
        h = _silu(h)
        out = jnp.einsum('bsf,fd->bsd', h, w2)
        return out
    x = A_x
    xn = _layernorm(x, axis=-1)
    return x + _A_ref(xn, A_mem0, A_Wq, A_Wk, A_Wv, A_Wo, A_seg_len) + _B_ref(xn, B_w1, B_w2)
```

```python
import functools

import jax
import jax.numpy as jnp
import jax.experimental.pallas as pl
import jax.experimental.pallas.tpu as pltpu

_F32 = jnp.float32
_BF16 = jnp.bfloat16
_LA = 8
_FFN_ROWS = 256


def _dot(a, b):
    return jnp.dot(a, b, preferred_element_type=_F32)


def _dot_nt(a, b):
    return jax.lax.dot_general(
        a, b, (((1,), (1,)), ((), ())), preferred_element_type=_F32)


def _kernel(
    xt_hbm,
    mem0_hbm,
    wq_hbm, wk_hbm, wv_hbm,
    wot_hbm,
    w1_hbm,
    w2t_hbm,
    outt_hbm,
    xt_s,
    xn_s,
    x_s,
    g_s,
    out_s,
    outt_s,
    mem0_s,
    wq_r, wk_r, wv_r,
    wot_r,
    wq_s, wk_s, wv_s,
    wo_s,
    w1_s, w2t_s,
    la_q, la_k, la_v,
    x_sems,
    in_sems,
    out_sem,
    *, S, Dm, H, Dh, M, seg, F,
):
    L = seg + M
    scale = Dh ** (-0.5)
    n_chunks = S // _FFN_ROWS

    def cp(src, dst, i):
        return pltpu.make_async_copy(src, dst, in_sems.at[i])

    def cp_x(c):
        return pltpu.make_async_copy(
            xt_hbm.at[:, pl.ds(c * _FFN_ROWS, _FFN_ROWS)], xt_s.at[c], x_sems.at[c])

    c_w1 = cp(w1_hbm, w1_s, 0)
    c_wq, c_wk, c_wv = cp(wq_hbm, wq_r, 2), cp(wk_hbm, wk_r, 3), cp(wv_hbm, wv_r, 4)
    c_wo = cp(wot_hbm, wot_r, 5)
    late = [cp(w2t_hbm, w2t_s, 1), cp(mem0_hbm, mem0_s, 6)]
    cp_x(0).start()
    c_w1.start()
    for c in range(1, n_chunks):
        cp_x(c).start()
    for c in [c_wq, c_wk, c_wv, c_wo] + late:
        c.start()

    grp = 16

    def relayout_qkv(copy, raw, dst):
        copy.wait()
        for gi in range(Dm // grp):
            v = jnp.swapaxes(raw[gi * grp:(gi + 1) * grp], 0, 1)
            for h in range(H):
                dst[gi * grp:(gi + 1) * grp, h * Dh:(h + 1) * Dh] = v[h]

    def layernorm_chunk(c):
        cp_x(c).wait()
        rows = slice(c * _FFN_ROWS, (c + 1) * _FFN_ROWS)
        xc = xt_s[c].astype(_F32).T
        mu = jnp.mean(xc, axis=-1, keepdims=True)
        xd = xc - mu
        var = jnp.mean(xd * xd, axis=-1, keepdims=True)
        xn_s[rows, :] = (xd * jax.lax.rsqrt(var + 1e-5)).astype(_BF16)
        x_s[rows, :] = xc.astype(_BF16)

    relayout_at = {(3 * n_chunks) // 8: (c_wq, wq_r, wq_s),
                   n_chunks // 2: (c_wk, wk_r, wk_s),
                   (3 * n_chunks) // 4: (c_wv, wv_r, wv_s)}
    layernorm_chunk(0)
    c_w1.wait()
    for c in range(n_chunks):
        rows = slice(c * _FFN_ROWS, (c + 1) * _FFN_ROWS)
        h1 = _dot(xn_s[rows, :], w1_s[...])
        g_s[rows, :] = (h1 * jax.nn.sigmoid(h1)).astype(_BF16)
        if c + 1 < n_chunks:
            layernorm_chunk(c + 1)
        if c in relayout_at:
            relayout_qkv(*relayout_at[c])

    c_wo.wait()
    for h in range(H):
        wo_s[h * Dh:(h + 1) * Dh, :] = wot_r[h].T
    for c in late:
        c.wait()

    ri = jax.lax.broadcasted_iota(jnp.int32, (L, L), 0)
    ci = jax.lax.broadcasted_iota(jnp.int32, (L, L), 1)
    allowed = (ri >= seg) | (ci >= seg) | (ci <= ri)

    head_cols = [slice(h * Dh, (h + 1) * Dh) for h in range(H)]

    def attend_all(q, k, v, filler):
        qb, kb, vb = q.astype(_BF16), k.astype(_BF16), v.astype(_BF16)
        ss = [jnp.where(allowed, _dot_nt(qb[:, c], kb[:, c]) * scale, -1e9)
              for c in head_cols]
        extra = filler()
        ms = [jnp.max(s, axis=-1, keepdims=True) for s in ss]
        es = [jnp.exp(s - m) for s, m in zip(ss, ms)]
        ls = [jnp.sum(e, axis=-1, keepdims=True) for e in es]
        ps = [(e / l).astype(_BF16) for e, l in zip(es, ls)]
        o = jnp.concatenate(
            [_dot(p, vb[:, c]) for p, c in zip(ps, head_cols)], axis=1)
        return o, extra

    def run_segment(lhs, first_of_pair, filler):
        q = _dot(lhs, wq_s[...])
        k = _dot(lhs, wk_s[...])
        v = _dot(lhs, wv_s[...])
        if first_of_pair:
            la_q[...] = q[L:L + _LA]
            la_k[...] = k[L:L + _LA]
            la_v[...] = v[L:L + _LA]
            q, k, v = q[:L], k[:L], v[:L]
        else:
            q = jnp.concatenate([la_q[...], q], axis=0)
            k = jnp.concatenate([la_k[...], k], axis=0)
            v = jnp.concatenate([la_v[...], v], axis=0)
        return attend_all(q, k, v, filler)

    n0 = seg - _LA

    def pair_body(j, mem):
        r0 = pl.multiple_of(j * (2 * seg), 2 * seg)
        x0 = xn_s[pl.ds(r0, seg), :]
        x1f = xn_s[pl.ds(r0 + seg, seg), :].astype(_F32)
        g = g_s[pl.ds(r0, 2 * seg), :]
        fh = F // 2
        tail = jnp.concatenate([mem, x1f[:_LA]], axis=0).astype(_BF16)
        lhs0 = jnp.concatenate([x0, tail], axis=0)
        o0, f0 = run_segment(lhs0, True, lambda: _dot_nt(g[:, :fh], w2t_s[:, :fh]))
        w0 = jnp.concatenate([o0[:n0], o0[seg:L]], axis=0).astype(_BF16)
        a0 = _dot(w0, wo_s[...])
        mem1 = a0[n0:n0 + M]
        lhs1 = jnp.concatenate([x1f[_LA:], mem1], axis=0).astype(_BF16)
        o1, f1 = run_segment(lhs1, False, lambda: _dot_nt(g[:, fh:], w2t_s[:, fh:]))
        w1r = jnp.concatenate([o1, o0[n0:seg]], axis=0).astype(_BF16)
        a1 = _dot(w1r, wo_s[...])
        attn = jnp.concatenate([a0[:n0], a1[L:L + _LA], a1[:seg]], axis=0)
        out_s[pl.ds(r0, 2 * seg), :] = (
            x_s[pl.ds(r0, 2 * seg), :].astype(_F32) + attn + (f0 + f1)).astype(_BF16)
        return a1[seg:L]

    pairs_per_group = _FFN_ROWS // (2 * seg)

    def group_body(g, mem):
        mem = jax.lax.fori_loop(
            g * pairs_per_group, (g + 1) * pairs_per_group, pair_body, mem)
        r0 = pl.multiple_of(g * _FFN_ROWS, _FFN_ROWS)
        outt_s[:, pl.ds(r0, _FFN_ROWS)] = out_s[pl.ds(r0, _FFN_ROWS), :].T
        pltpu.make_async_copy(
            outt_s.at[:, pl.ds(r0, _FFN_ROWS)], outt_hbm.at[:, pl.ds(r0, _FFN_ROWS)],
            out_sem).start()
        return mem

    jax.lax.fori_loop(0, S // _FFN_ROWS, group_body, mem0_s[...].astype(_F32))

    pltpu.make_async_copy(outt_s, outt_hbm, out_sem).wait()


@functools.partial(jax.jit, static_argnames=("A_seg_len",))
def pallas_parallel_sum__memory_aug_recurrent_mem_tr__dense_activation_silu__prompt_kernel(
    A_x: jax.Array,
    A_mem0: jax.Array,
    A_Wq: jax.Array,
    A_Wk: jax.Array,
    A_Wv: jax.Array,
    A_Wo: jax.Array,
    A_seg_len,
    B_x: jax.Array,
    B_w1: jax.Array,
    B_w2: jax.Array,
):
    B, S, Dm = A_x.shape
    H, Dh = A_Wq.shape[1], A_Wq.shape[2]
    M = A_mem0.shape[1]
    F = B_w1.shape[1]
    HD = H * Dh
    seg = int(A_seg_len)
    assert B == 1 and S % (2 * seg) == 0 and S % _FFN_ROWS == 0
    assert seg % 16 == 0 and M == _LA and (seg + M + _LA) % 16 == 0

    kernel = functools.partial(
        _kernel, S=S, Dm=Dm, H=H, Dh=Dh, M=M, seg=seg, F=F)

    any_spec = pl.BlockSpec(memory_space=pl.ANY)
    n_chunks = S // _FFN_ROWS
    assert n_chunks % 8 == 0 and Dm % 16 == 0
    assert _FFN_ROWS % (2 * seg) == 0
    assert F % 256 == 0
    outt = pl.pallas_call(
        kernel,
        out_shape=jax.ShapeDtypeStruct((Dm, S), _BF16),
        in_specs=[any_spec] * 8,
        out_specs=any_spec,
        scratch_shapes=[
            pltpu.VMEM((n_chunks, Dm, _FFN_ROWS), _BF16),
            pltpu.VMEM((S, Dm), _BF16),
            pltpu.VMEM((S, Dm), _BF16),
            pltpu.VMEM((S, F), _BF16),
            pltpu.VMEM((S, Dm), _BF16),
            pltpu.VMEM((Dm, S), _BF16),
            pltpu.VMEM((M, Dm), _BF16),
            pltpu.VMEM((Dm, H, Dh), _BF16),
            pltpu.VMEM((Dm, H, Dh), _BF16),
            pltpu.VMEM((Dm, H, Dh), _BF16),
            pltpu.VMEM((H, Dm, Dh), _BF16),
            pltpu.VMEM((Dm, HD), _BF16),
            pltpu.VMEM((Dm, HD), _BF16),
            pltpu.VMEM((Dm, HD), _BF16),
            pltpu.VMEM((HD, Dm), _BF16),
            pltpu.VMEM((Dm, F), _BF16),
            pltpu.VMEM((Dm, F), _BF16),
            pltpu.VMEM((_LA, HD), _F32),
            pltpu.VMEM((_LA, HD), _F32),
            pltpu.VMEM((_LA, HD), _F32),
            pltpu.SemaphoreType.DMA((n_chunks,)),
            pltpu.SemaphoreType.DMA((7,)),
            pltpu.SemaphoreType.DMA(()),
        ],
        compiler_params=pltpu.CompilerParams(
            vmem_limit_bytes=100 * 1024 * 1024),
    )(
        jnp.swapaxes(A_x, 1, 2).reshape(Dm, S),
        A_mem0.reshape(M, Dm),
        A_Wq,
        A_Wk,
        A_Wv,
        jnp.swapaxes(A_Wo, 1, 2),
        B_w1,
        B_w2.T,
    )
    return jnp.swapaxes(outt.reshape(B, Dm, S), 1, 2)
```
